```python
import os as _os
_os.environ.setdefault("JAX_PLATFORMS", "cpu")
import jax
import jax.numpy as jnp

def _softmax(x, axis=-1):
    return jax.nn.softmax(x, axis=axis)
def _gelu(x):
    return jax.nn.gelu(x, approximate=True)
def _silu(x):
    return jax.nn.silu(x)
def _sigmoid(x):
    return jax.nn.sigmoid(x)
def _layernorm(x, axis=-1, eps=1e-5):
    m = jnp.mean(x, axis=axis, keepdims=True)
    v = jnp.var(x, axis=axis, keepdims=True)
    return (x - m) / jnp.sqrt(v + eps)
def _scatter_add(tgt, idx, src, axis=0):
    return tgt.at[idx].add(src)
def _segment_sum(src, seg, n):
    return jax.ops.segment_sum(src, seg, n)
class _Rng:
    def __init__(self, key):
        self._k = key
    def _next(self):
        self._k, sub = jax.random.split(self._k)
        return sub
    def normal(self, shape):
        return jax.random.normal(self._next(), shape, dtype=jnp.bfloat16)
    def randint(self, lo, hi, shape):
        return jax.random.randint(self._next(), shape, lo, hi, dtype=jnp.int32)
    def uniform(self, shape, lo=0.0, hi=1.0):
        return jax.random.uniform(self._next(), shape, jnp.bfloat16, lo, hi)
    def permutation(self, n):
        return jax.random.permutation(self._next(), n)


kernel_name = 'standalone__groupnorm__sampling'

def setup_inputs():
    _rng = _Rng(jax.random.key(int.from_bytes(__import__("os").urandom(4), "little")))
    _w = (lambda a: (lambda t: t.astype(jnp.bfloat16) if jnp.issubdtype(t.dtype, jnp.floating) else t)(jnp.asarray(a)))
    B = 32
    G = 32
    cpg = max(1, 576 // G)
    C = G * cpg
    H, W = 32, 16
    return {
        "x": _w((lambda *s: _rng.normal(s) * 0.05)(B, C, H, W)),
        "g": _w((lambda *s: _rng.normal(s) * 0.05)(C) + 1.0),
        "b": _w((lambda *s: _rng.normal(s) * 0.05)(C)),
    }

def reference(x, g, b):
    G = 32
    B, C, H, W = x.shape[0], x.shape[1], x.shape[2], x.shape[3]
    xr = x.reshape(B, G, C // G, H, W)
    mu = xr.mean(axis=(2, 3, 4), keepdims=True)
    var = ((xr - mu) ** 2).mean(axis=(2, 3, 4), keepdims=True)
    xn = (xr - mu) / jnp.sqrt(var + 1e-5)
    xn = xn.reshape(B, C, H, W)
    return xn * g[None, :, None, None] + b[None, :, None, None]
```

```python
import jax
import jax.numpy as jnp
from jax import lax
import jax.experimental.pallas as pl
import jax.experimental.pallas.tpu as pltpu

NUM_GROUPS = 32
EPS = 1e-5

STREAMS = 8
DMA_ROWS = 16
READ_LEAD = 8
WRITE_LEAD = 8
READ_TAIL = 5
UNITS_PER_SAMPLE = (1, 2, 2)
ROWS = 16


def _group_allreduce(v, width):
  lanes = v.shape[1]
  pos = lax.broadcasted_iota(jnp.int32, v.shape, 1) % width

  def rotate(a, k):
    return jnp.where(
        pos < width - k, pltpu.roll(a, lanes - k, 1), pltpu.roll(a, width - k, 1)
    )

  span, factor = width, 2
  while span > 1:
    if span % factor:
      factor += 1
      continue
    span //= factor
    total = v
    for i in range(1, factor):
      total = total + rotate(v, i * span)
    v = total
  return v


def _kernel(x_hbm, g_hbm, b_hbm, o_hbm, x_buf, o_buf, g_buf, b_buf, sum_ref,
            mean_ref, scale_ref, read_sem, write_sem, param_sem):
  batch, hw, c = x_hbm.shape
  width = c // NUM_GROUPS
  count = width * hw
  blocks = batch // STREAMS
  early_blocks = blocks // 2
  block_units = hw // DMA_ROWS
  units = blocks * block_units
  math_units = sum(UNITS_PER_SAMPLE) * STREAMS
  assert batch % STREAMS == 0 and hw % DMA_ROWS == 0 and hw % ROWS == 0
  assert block_units + READ_LEAD + early_blocks * math_units <= units
  for i in range(blocks - early_blocks):
    assert WRITE_LEAD + (i + 1) * math_units <= (early_blocks + i) * block_units

  def locate(unit):
    if isinstance(unit, int):
      block, step = divmod(unit, block_units)
      return block, pl.ds(step * DMA_ROWS, DMA_ROWS)
    row = pl.multiple_of(lax.rem(unit, block_units) * DMA_ROWS, DMA_ROWS)
    return lax.div(unit, block_units), pl.ds(row, DMA_ROWS)

  def start_read(unit):
    block, rows = locate(unit)
    sem = read_sem.at[
        block if isinstance(unit, int)
        else jnp.where(unit >= units - READ_TAIL, blocks, block)
    ]
    for k in range(STREAMS):
      s = block * STREAMS + k
      pltpu.make_async_copy(x_hbm.at[s, rows], x_buf.at[s, rows], sem).start(
          priority=k % 2)

  def start_write(unit):
    block, rows = locate(unit)
    for k in range(STREAMS):
      s = block * STREAMS + k
      pltpu.make_async_copy(
          o_buf.at[s, rows], o_hbm.at[s, rows], write_sem
      ).start(priority=k % 2)

  def wait_reads(block, rows, sem):
    idx = (pl.ds(block * STREAMS, STREAMS), rows)
    pltpu.make_async_copy(x_hbm.at[idx], x_buf.at[idx], read_sem.at[sem]).wait()

  def start_range(start, lo, hi):
    lax.fori_loop(lo, hi, lambda unit, _: start(unit), None)

  g_copy = pltpu.make_async_copy(g_hbm, g_buf, param_sem.at[0])
  b_copy = pltpu.make_async_copy(b_hbm, b_buf, param_sem.at[1])
  start_read(0)
  g_copy.start()
  b_copy.start()
  start_range(start_read, 1, block_units + READ_LEAD)
  sum_ref[...] = jnp.zeros_like(sum_ref)
  g_copy.wait()
  b_copy.wait()
  gamma = g_buf[...].astype(jnp.float32).reshape(1, c)
  beta = b_buf[...].astype(jnp.float32).reshape(1, c)

  def load(s, r):
    return x_buf[s, pl.ds(r, ROWS), :].astype(jnp.float32)

  def stat_row(ref, k, rows):
    return jnp.broadcast_to(ref[pl.ds(k, 1), pl.ds(0, c)], (rows, c))

  def normalise(block, issue):
    def for_each_sample(which, body):
      first = sum(UNITS_PER_SAMPLE[:which]) * STREAMS
      per_sample = UNITS_PER_SAMPLE[which]

      def step(k, _):
        for i in range(per_sample):
          issue(first + k * per_sample + i)
        body(k, block * STREAMS + k)

      lax.fori_loop(0, STREAMS, step, None)

    def channel_sums(k, s, term):
      acc = jnp.zeros((8, c), jnp.float32)
      for r in range(0, hw, ROWS):
        v = load(s, r)
        for q in range(0, ROWS, 8):
          acc = acc + term(v[q:q + 8])
      sum_ref[pl.ds(k, 1), pl.ds(0, c)] = jnp.sum(acc, axis=0, keepdims=True)

    def sum_values(k, s):
      channel_sums(k, s, lambda v: v)

    def sum_squared_deviations(k, s):
      mean = stat_row(mean_ref, k, 8)
      channel_sums(k, s, lambda v: (v - mean) * (v - mean))

    def scale_and_shift(k, s):
      mean = stat_row(mean_ref, k, ROWS)
      scale = stat_row(scale_ref, k, ROWS)
      shift = jnp.broadcast_to(beta, (ROWS, c))
      for r in range(0, hw, ROWS):
        y = (load(s, r) - mean) * scale + shift
        o_buf[s, pl.ds(r, ROWS), :] = y.astype(o_buf.dtype)

    for_each_sample(0, sum_values)
    mean_ref[...] = _group_allreduce(sum_ref[...], width) / count
    for_each_sample(1, sum_squared_deviations)
    var = _group_allreduce(sum_ref[...], width) / count
    scale_ref[...] = lax.rsqrt(var[:, :c] + EPS) * gamma
    for_each_sample(2, scale_and_shift)

  def finish_reads_and_start_writes():
    start_range(
        start_read, block_units + READ_LEAD + early_blocks * math_units, units)
    for block in range(early_blocks, blocks - 1):
      wait_reads(block, pl.ds(0, hw), block)
    tail = READ_TAIL * DMA_ROWS
    wait_reads(blocks - 1, pl.ds(0, hw - tail), blocks - 1)
    start_range(start_write, 0, WRITE_LEAD)
    wait_reads(blocks - 1, pl.ds(hw - tail, tail), blocks)

  def block_step(block, _):
    reading = block < early_blocks
    pl.when(reading)(lambda: wait_reads(block, pl.ds(0, hw), block))
    pl.when(block == early_blocks)(finish_reads_and_start_writes)

    def issue(i):
      pl.when(reading)(
          lambda: start_read(block_units + READ_LEAD + block * math_units + i))
      pl.when(block >= early_blocks)(
          lambda: start_write(
              WRITE_LEAD + (block - early_blocks) * math_units + i))

    normalise(block, issue)

  lax.fori_loop(0, blocks, block_step, None)
  start_range(
      start_write, WRITE_LEAD + (blocks - early_blocks) * math_units, units)
  pltpu.make_async_copy(o_buf, o_hbm, write_sem).wait()


@jax.jit
def pallas_standalone__groupnorm__sampling_kernel(
    x: jax.Array,
    g: jax.Array,
    b: jax.Array,
):
  batch, c, h, w = x.shape
  shape = (batch, h * w, c)
  stats_shape = (STREAMS, pl.cdiv(c, 128) * 128)
  hbm = pl.BlockSpec(memory_space=pltpu.HBM)
  out = pl.pallas_call(
      _kernel,
      in_specs=[hbm, hbm, hbm],
      out_specs=hbm,
      out_shape=jax.ShapeDtypeStruct(shape, x.dtype),
      scratch_shapes=[
          pltpu.VMEM(shape, x.dtype),
          pltpu.VMEM(shape, x.dtype),
          pltpu.VMEM((c,), g.dtype),
          pltpu.VMEM((c,), b.dtype),
          pltpu.VMEM(stats_shape, jnp.float32),
          pltpu.VMEM(stats_shape, jnp.float32),
          pltpu.VMEM((STREAMS, c), jnp.float32),
          pltpu.SemaphoreType.DMA((batch // STREAMS + 1,)),
          pltpu.SemaphoreType.DMA(()),
          pltpu.SemaphoreType.DMA((2,)),
      ],
      compiler_params=pltpu.CompilerParams(
          vmem_limit_bytes=64 * 1024 * 1024,
          disable_bounds_checks=True,
          disable_semaphore_checks=True,
      ),
      name="groupnorm",
  )(jnp.transpose(x, (0, 2, 3, 1)).reshape(shape), g, b)
  return jnp.transpose(out.reshape(batch, h, w, c), (0, 3, 1, 2))
```

```python
import jax
import jax.numpy as jnp
from jax import lax
import jax.experimental.pallas as pl
import jax.experimental.pallas.tpu as pltpu

NUM_GROUPS = 32
EPS = 1e-5

STREAMS = 8
STREAM_ORDER = (0, 1, 4, 5, 2, 3, 6, 7)
DMA_ROWS = 16
READ_LEAD = 8
WRITE_LEAD = 8
READ_TAIL = 5
UNITS_PER_SAMPLE = (1, 2, 2)
ROWS = 16


def _group_allreduce(v, width):
  lanes = v.shape[1]
  pos = lax.broadcasted_iota(jnp.int32, v.shape, 1) % width

  def rotate(a, k):
    return jnp.where(
        pos < width - k, pltpu.roll(a, lanes - k, 1), pltpu.roll(a, width - k, 1)
    )

  span, factor = width, 2
  while span > 1:
    if span % factor:
      factor += 1
      continue
    span //= factor
    total = v
    for i in range(1, factor):
      total = total + rotate(v, i * span)
    v = total
  return v


def _kernel(x_hbm, g_hbm, b_hbm, o_hbm, x_buf, o_buf, g_buf, b_buf, sum_ref,
            mean_ref, scale_ref, read_sem, write_sem, param_sem):
  batch, hw, c = x_hbm.shape
  width = c // NUM_GROUPS
  count = width * hw
  blocks = batch // STREAMS
  early_blocks = blocks // 2
  block_units = hw // DMA_ROWS
  units = blocks * block_units
  math_units = sum(UNITS_PER_SAMPLE) * STREAMS
  assert sorted(STREAM_ORDER) == list(range(STREAMS))
  assert c % NUM_GROUPS == 0 and batch % STREAMS == 0
  assert hw % DMA_ROWS == 0 and hw % ROWS == 0
  assert block_units + READ_LEAD + early_blocks * math_units <= units
  for i in range(blocks - early_blocks):
    assert WRITE_LEAD + (i + 1) * math_units <= (early_blocks + i) * block_units

  def locate(unit):
    if isinstance(unit, int):
      block, step = divmod(unit, block_units)
      return block, pl.ds(step * DMA_ROWS, DMA_ROWS)
    row = pl.multiple_of(lax.rem(unit, block_units) * DMA_ROWS, DMA_ROWS)
    return lax.div(unit, block_units), pl.ds(row, DMA_ROWS)

  def start_read(unit):
    block, rows = locate(unit)
    sem = read_sem.at[
        block if isinstance(unit, int)
        else jnp.where(unit >= units - READ_TAIL, blocks, block)
    ]
    for i, k in enumerate(STREAM_ORDER):
      s = block * STREAMS + k
      pltpu.make_async_copy(x_hbm.at[s, rows], x_buf.at[s, rows], sem).start(
          priority=i % 2)

  def start_write(unit):
    block, rows = locate(unit)
    for i, k in enumerate(STREAM_ORDER):
      s = block * STREAMS + k
      pltpu.make_async_copy(
          o_buf.at[s, rows], o_hbm.at[s, rows], write_sem
      ).start(priority=1 - i % 2)

  def wait_reads(block, rows, sem):
    idx = (pl.ds(block * STREAMS, STREAMS), rows)
    pltpu.make_async_copy(x_hbm.at[idx], x_buf.at[idx], read_sem.at[sem]).wait()

  def start_range(start, lo, hi):
    lax.fori_loop(lo, hi, lambda unit, _: start(unit), None)

  g_copy = pltpu.make_async_copy(g_hbm, g_buf, param_sem.at[0])
  b_copy = pltpu.make_async_copy(b_hbm, b_buf, param_sem.at[1])
  start_read(0)
  g_copy.start()
  b_copy.start()
  start_range(start_read, 1, block_units + READ_LEAD)
  sum_ref[...] = jnp.zeros_like(sum_ref)
  g_copy.wait()
  b_copy.wait()
  gamma = g_buf[...].astype(jnp.float32).reshape(1, c)
  beta = b_buf[...].astype(jnp.float32).reshape(1, c)

  def load(s, r):
    return x_buf[s, pl.ds(r, ROWS), :].astype(jnp.float32)

  def stat_row(ref, k, rows):
    return jnp.broadcast_to(ref[pl.ds(k, 1), pl.ds(0, c)], (rows, c))

  def normalise(block, issue):
    def for_each_sample(which, body):
      first = sum(UNITS_PER_SAMPLE[:which]) * STREAMS
      per_sample = UNITS_PER_SAMPLE[which]

      def step(k, _):
        for i in range(per_sample):
          issue(first + k * per_sample + i)
        body(k, block * STREAMS + k)

      lax.fori_loop(0, STREAMS, step, None)

    def channel_sums(k, s, term):
      acc = jnp.zeros((8, c), jnp.float32)
      for r in range(0, hw, ROWS):
        v = load(s, r)
        for q in range(0, ROWS, 8):
          acc = acc + term(v[q:q + 8])
      sum_ref[pl.ds(k, 1), pl.ds(0, c)] = jnp.sum(acc, axis=0, keepdims=True)

    def sum_values(k, s):
      channel_sums(k, s, lambda v: v)

    def sum_squared_deviations(k, s):
      mean = stat_row(mean_ref, k, 8)
      channel_sums(k, s, lambda v: (v - mean) * (v - mean))

    def scale_and_shift(k, s):
      mean = stat_row(mean_ref, k, ROWS)
      scale = stat_row(scale_ref, k, ROWS)
      shift = jnp.broadcast_to(beta, (ROWS, c))
      for r in range(0, hw, ROWS):
        y = (load(s, r) - mean) * scale + shift
        o_buf[s, pl.ds(r, ROWS), :] = y.astype(o_buf.dtype)

    for_each_sample(0, sum_values)
    mean_ref[...] = _group_allreduce(sum_ref[...], width) / count
    for_each_sample(1, sum_squared_deviations)
    var = _group_allreduce(sum_ref[...], width) / count
    scale_ref[...] = lax.rsqrt(var[:, :c] + EPS) * gamma
    for_each_sample(2, scale_and_shift)

  def finish_reads_and_start_writes():
    start_range(
        start_read, block_units + READ_LEAD + early_blocks * math_units, units)
    for block in range(early_blocks, blocks - 1):
      wait_reads(block, pl.ds(0, hw), block)
    tail = READ_TAIL * DMA_ROWS
    wait_reads(blocks - 1, pl.ds(0, hw - tail), blocks - 1)
    start_range(start_write, 0, WRITE_LEAD)
    wait_reads(blocks - 1, pl.ds(hw - tail, tail), blocks)

  def block_step(block, _):
    reading = block < early_blocks
    pl.when(reading)(lambda: wait_reads(block, pl.ds(0, hw), block))
    pl.when(block == early_blocks)(finish_reads_and_start_writes)

    def issue(i):
      pl.when(reading)(
          lambda: start_read(block_units + READ_LEAD + block * math_units + i))
      pl.when(block >= early_blocks)(
          lambda: start_write(
              WRITE_LEAD + (block - early_blocks) * math_units + i))

    normalise(block, issue)

  lax.fori_loop(0, blocks, block_step, None)
  start_range(
      start_write, WRITE_LEAD + (blocks - early_blocks) * math_units, units)
  pltpu.make_async_copy(o_buf, o_hbm, write_sem).wait()


@jax.jit
def pallas_standalone__groupnorm__sampling_kernel(
    x: jax.Array,
    g: jax.Array,
    b: jax.Array,
):
  batch, c, h, w = x.shape
  shape = (batch, h * w, c)
  stats_shape = (STREAMS, pl.cdiv(c, 128) * 128)
  hbm = pl.BlockSpec(memory_space=pltpu.HBM)
  out = pl.pallas_call(
      _kernel,
      in_specs=[hbm, hbm, hbm],
      out_specs=hbm,
      out_shape=jax.ShapeDtypeStruct(shape, x.dtype),
      scratch_shapes=[
          pltpu.VMEM(shape, x.dtype),
          pltpu.VMEM(shape, x.dtype),
          pltpu.VMEM((c,), g.dtype),
          pltpu.VMEM((c,), b.dtype),
          pltpu.VMEM(stats_shape, jnp.float32),
          pltpu.VMEM(stats_shape, jnp.float32),
          pltpu.VMEM((STREAMS, c), jnp.float32),
          pltpu.SemaphoreType.DMA((batch // STREAMS + 1,)),
          pltpu.SemaphoreType.DMA(()),
          pltpu.SemaphoreType.DMA((2,)),
      ],
      compiler_params=pltpu.CompilerParams(
          vmem_limit_bytes=64 * 1024 * 1024,
          disable_bounds_checks=True,
          disable_semaphore_checks=True,
      ),
      name="groupnorm",
  )(jnp.transpose(x, (0, 2, 3, 1)).reshape(shape), g, b)
  return jnp.transpose(out.reshape(batch, h, w, c), (0, 3, 1, 2))
```
